```python
import os as _os
_os.environ.setdefault("JAX_PLATFORMS", "cpu")
import jax
import jax.numpy as jnp

def _softmax(x, axis=-1):
    return jax.nn.softmax(x, axis=axis)
def _gelu(x):
    return jax.nn.gelu(x, approximate=True)
def _silu(x):
    return jax.nn.silu(x)
def _sigmoid(x):
    return jax.nn.sigmoid(x)
def _layernorm(x, axis=-1, eps=1e-5):
    m = jnp.mean(x, axis=axis, keepdims=True)
    v = jnp.var(x, axis=axis, keepdims=True)
    return (x - m) / jnp.sqrt(v + eps)
def _scatter_add(tgt, idx, src, axis=0):
    return tgt.at[idx].add(src)
def _segment_sum(src, seg, n):
    return jax.ops.segment_sum(src, seg, n)
class _Rng:
    def __init__(self, key):
        self._k = key
    def _next(self):
        self._k, sub = jax.random.split(self._k)
        return sub
    def normal(self, shape):
        return jax.random.normal(self._next(), shape, dtype=jnp.bfloat16)
    def randint(self, lo, hi, shape):
        return jax.random.randint(self._next(), shape, lo, hi, dtype=jnp.int32)
    def uniform(self, shape, lo=0.0, hi=1.0):
        return jax.random.uniform(self._next(), shape, jnp.bfloat16, lo, hi)
    def permutation(self, n):
        return jax.random.permutation(self._next(), n)


kernel_name = 'concat_heads__mha_block_cached__mha_block_cached__near_ridge'

def setup_inputs():
    _rng = _Rng(jax.random.key(int.from_bytes(__import__("os").urandom(4), "little")))
    _w = (lambda a: (lambda t: t.astype(jnp.bfloat16) if jnp.issubdtype(t.dtype, jnp.floating) else t)(jnp.asarray(a)))
    def _A_setup():
        B, Sq, D = 8, 160, 512
        H, Sk, Dh = 32, 512, 128
        return {
            "x": _w((lambda *s: _rng.normal(s) * 0.8)(B, Sq, D)),
            "k_cache": _w((lambda *s: _rng.normal(s) * 0.8)(B, H, Sk, Dh)),
            "v_cache": _w((lambda *s: _rng.normal(s) * 0.05)(B, H, Sk, Dh)),
            "wq": _w((lambda *s: _rng.normal(s) * 0.8)(D, H * Dh) * (D ** -0.5)),
            "wo": _w((lambda *s: _rng.normal(s) * 0.05)(H * Dh, D) * ((H * Dh) ** -0.5)),
        }
    _A_in = _A_setup()

    def _B_setup():
        B, Sq, D = 8, 160, 512
        H, Sk, Dh = 32, 512, 128
        return {
            "x": _w((lambda *s: _rng.normal(s) * 0.8)(B, Sq, D)),
            "k_cache": _w((lambda *s: _rng.normal(s) * 0.8)(B, H, Sk, Dh)),
            "v_cache": _w((lambda *s: _rng.normal(s) * 0.05)(B, H, Sk, Dh)),
            "wq": _w((lambda *s: _rng.normal(s) * 0.8)(D, H * Dh) * (D ** -0.5)),
            "wo": _w((lambda *s: _rng.normal(s) * 0.05)(H * Dh, D) * ((H * Dh) ** -0.5)),
        }
    _B_in = _B_setup()

    return {
        "A_x": _A_in["x"],
        "A_k_cache": _A_in["k_cache"],
        "A_v_cache": _A_in["v_cache"],
        "A_wq": _A_in["wq"],
        "A_wo": _A_in["wo"],
        "B_x": _B_in["x"],
        "B_k_cache": _B_in["k_cache"],
        "B_v_cache": _B_in["v_cache"],
        "B_wq": _B_in["wq"],
        "B_wo": _B_in["wo"],
    }

def reference(A_x, A_k_cache, A_v_cache, A_wq, A_wo, B_x, B_k_cache, B_v_cache, B_wq, B_wo):
    def _A_ref(x, k_cache, v_cache, wq, wo):
        B, Sq, D = x.shape
        H, Dh = 32, 128
        q = (lambda x, *d: x.transpose(*d))((x @ wq).reshape(B, Sq, H, Dh), 0, 2, 1, 3)
        scores = jnp.einsum("bhqd,bhkd->bhqk", q, k_cache) * (Dh ** -0.5)
        p = _softmax(scores, axis=-1)
        o = jnp.einsum("bhqk,bhkd->bhqd", p, v_cache)
        return (lambda x, *d: x.transpose(*d))(o, 0, 2, 1, 3).reshape(B, Sq, H * Dh) @ wo

    def _B_ref(x, k_cache, v_cache, wq, wo):
        B, Sq, D = x.shape
        H, Dh = 32, 128
        q = (lambda x, *d: x.transpose(*d))((x @ wq).reshape(B, Sq, H, Dh), 0, 2, 1, 3)
        scores = jnp.einsum("bhqd,bhkd->bhqk", q, k_cache) * (Dh ** -0.5)
        p = _softmax(scores, axis=-1)
        o = jnp.einsum("bhqk,bhkd->bhqd", p, v_cache)
        return (lambda x, *d: x.transpose(*d))(o, 0, 2, 1, 3).reshape(B, Sq, H * Dh) @ wo

    a = _A_ref(A_x, A_k_cache, A_v_cache, A_wq, A_wo)
    b = _B_ref(B_x, B_k_cache, B_v_cache, B_wq, B_wo)
    return jnp.concatenate([a, b], axis=-1)
```

```python
import jax
import jax.numpy as jnp
from jax import lax
import jax.experimental.pallas as pl
import jax.experimental.pallas.tpu as pltpu

B, Sq, D, H, Sk, Dh = 8, 160, 512, 32, 512, 128
LOG2E = 1.4426950408889634
SCALE = Dh ** -0.5
f32 = jnp.float32; bf16 = jnp.bfloat16

def make_v4(nb=4, nh=4, NB=3, vmem=100, dbg_kv=None, nobounds=True, OG=4):
    NHG = H // nh; NBG = B // nb
    SPB = NHG * NBG
    S = 2 * SPB
    assert nh % OG == 0
    def kernel(ax, ak, av, awq, awo, bx, bk, bv, bwq, bwo, out_hbm,
               x_buf, k_buf, v_buf, wq_buf, wo_buf, acc, out_buf,
               x_sem, kv_sem, w_sem, o_sem):
        s = pl.program_id(0)
        def decode(t):
            blk = t // SPB; r = t % SPB
            return blk, r // NBG, r % NBG
        def kv_copies(kh, vh, t, slot):
            _, hg, bg = decode(t)
            cps = [pltpu.make_async_copy(kh.at[pl.ds(bg * nb, nb), pl.ds(hg * nh, nh)], k_buf.at[slot], kv_sem.at[slot]),
                   pltpu.make_async_copy(vh.at[pl.ds(bg * nb, nb), pl.ds(hg * nh, nh)], v_buf.at[slot], kv_sem.at[slot])]
            if dbg_kv is not None: cps = cps[:dbg_kv]
            return cps
        def start_kv(t, cond=True):
            slot = t % NB
            blk = t // SPB
            @pl.when((blk == 0) & cond)
            def _():
                for c in kv_copies(ak, av, t, slot): c.start()
            @pl.when((blk == 1) & cond)
            def _():
                for c in kv_copies(bk, bv, t, slot): c.start()
        def w_copies(wq, wo, w, wslot):
            hg = w % NHG
            return [pltpu.make_async_copy(wq.at[:, pl.ds(pl.multiple_of(hg * nh * Dh, Dh), nh * Dh)], wq_buf.at[wslot], w_sem.at[wslot]),
                    pltpu.make_async_copy(wo.at[pl.ds(pl.multiple_of(hg * nh * Dh, Dh), nh * Dh), :], wo_buf.at[wslot], w_sem.at[wslot])]
        def start_w(w, cond=True):
            wslot = w % 2
            @pl.when((w < NHG) & cond)
            def _():
                for c in w_copies(awq, awo, w, wslot): c.start()
            @pl.when((w >= NHG) & cond)
            def _():
                for c in w_copies(bwq, bwo, w, wslot): c.start()
        def x_copy(i, g):
            return pltpu.make_async_copy((ax, bx)[i].at[pl.ds(g * nb, nb)], x_buf.at[i, pl.ds(g * nb, nb)], x_sem.at[i * NBG + g])
        def once(fn):
            lax.fori_loop(0, jnp.minimum(s + 1, 1), lambda i, c: (fn(), c)[1], 0)

        blk, hg, bg = decode(s)
        w = s // NBG
        slot = s % NB
        wslot = w % 2

        @pl.when(s == 0)
        def _prologue():
            x_copy(0, 0).start()
            start_w(0)
            start_kv(0)
            def stage2():
                for g in range(1, NBG): x_copy(0, g).start()
                for t in range(1, NB - 1): start_kv(t)
            once(stage2)
            acc[...] = jnp.zeros_like(acc)

        @pl.when(s == min(1, SPB - 1))
        def _():
            for g in range(NBG): x_copy(1, g).start()
        for g in range(NBG):
            for i in range(2):
                @pl.when((hg == 0) & (bg == g) & (blk == i))
                def _():
                    x_copy(i, g).wait()
        start_w(w + 1, (bg == 0) & (w + 1 < 2 * NHG))
        start_kv(s + NB - 1, s + NB - 1 < S)
        @pl.when(bg == 0)
        def _():
            for c in w_copies(awq, awo, w, wslot): c.wait()
        for c in kv_copies(ak, av, s, slot): c.wait()

        last_hg = hg == NHG - 1
        def out_copy():
            return pltpu.make_async_copy(out_buf, out_hbm.at[pl.ds(bg * nb, nb), :, pl.ds(pl.multiple_of(blk * D, D), D)], o_sem)
        @pl.when(last_hg & ((bg > 0) | (blk == 1)))
        def _():
            out_copy().wait()

        units = [(bi, hi) for bi in range(nb) for hi in range(nh)]
        N = len(units)
        q, p, r, o, ocat = {}, {}, {}, {}, {}
        def Q(u):
            bi, hi = units[u]
            t = jnp.dot(x_buf[blk, bg * nb + bi], wq_buf[wslot, :, hi * Dh:(hi + 1) * Dh], preferred_element_type=f32)
            q[u] = (t * (SCALE * LOG2E)).astype(bf16)
        def Sx(u):
            bi, hi = units[u]
            sc = lax.dot_general(q.pop(u), k_buf[slot, bi, hi], (((1,), (1,)), ((), ())), preferred_element_type=f32)
            m = jnp.max(sc, axis=-1, keepdims=True)
            e = jnp.exp2(sc - m)
            l = jnp.sum(e, axis=-1, keepdims=True)
            p[u] = e.astype(bf16)
            rr = pl.reciprocal(l, approx=True)
            r[u] = rr * (2.0 - l * rr)
        def V(u):
            bi, hi = units[u]
            t = jnp.dot(p.pop(u), v_buf[slot, bi, hi], preferred_element_type=f32)
            o[u] = (t * r.pop(u)).astype(bf16)
        def O(grp, j):
            bi, h0 = units[grp]
            if grp not in ocat:
                ocat[grp] = jnp.concatenate([o.pop(grp + i) for i in range(OG)], axis=-1)
            y = jnp.dot(ocat[grp], wo_buf[wslot, h0 * Dh:(h0 + OG) * Dh, j * 128:(j + 1) * 128], preferred_element_type=f32)
            acc[blk, bg * nb + bi, :, j * 128:(j + 1) * 128] += y
        pend = []
        Q(0); Q(1)
        for u in range(N + 1):
            if u < N: Sx(u)
            ready = []
            if u >= 1:
                V(u - 1)
                if (u - 1) % OG == OG - 1:
                    ready = [(u - OG, j) for j in range(4)]
            if u + 2 < N: Q(u + 2)
            for _ in range(max(1, 4 // OG)):
                if pend: O(*pend.pop(0))
            pend += ready
        while pend: O(*pend.pop(0))

        @pl.when(last_hg)
        def _():
            for bi in range(nb):
                out_buf[bi] = acc[blk, bg * nb + bi].astype(bf16)
            out_copy().start()
        @pl.when(s == S - 1)
        def _():
            out_copy().wait()

    anys = pl.BlockSpec(memory_space=pl.ANY)
    @jax.jit
    def fn(*args):
        return pl.pallas_call(
            kernel, grid=(S,), in_specs=[anys] * 10, out_specs=anys,
            out_shape=jax.ShapeDtypeStruct((B, Sq, 2 * D), bf16),
            scratch_shapes=[
                pltpu.VMEM((2, B, Sq, D), bf16),
                pltpu.VMEM((NB, nb, nh, Sk, Dh), bf16),
                pltpu.VMEM((NB, nb, nh, Sk, Dh), bf16),
                pltpu.VMEM((2, D, nh * Dh), bf16),
                pltpu.VMEM((2, nh * Dh, D), bf16),
                pltpu.VMEM((2, B, Sq, D), f32),
                pltpu.VMEM((nb, Sq, D), bf16),
                pltpu.SemaphoreType.DMA((2 * NBG,)),
                pltpu.SemaphoreType.DMA((NB,)),
                pltpu.SemaphoreType.DMA((2,)),
                pltpu.SemaphoreType.DMA(()),
            ],
            compiler_params=pltpu.CompilerParams(dimension_semantics=("arbitrary",), vmem_limit_bytes=vmem * 1024 * 1024,
                                                 disable_bounds_checks=nobounds),
        )(*args)
    return fn


_impl = make_v4(4, 4, 3)


def pallas_concat_heads__mha_block_cached__mha_block_cached__near_ridge_kernel(
    A_x, A_k_cache, A_v_cache, A_wq, A_wo, B_x, B_k_cache, B_v_cache, B_wq, B_wo
):
    return _impl(A_x, A_k_cache, A_v_cache, A_wq, A_wo, B_x, B_k_cache, B_v_cache, B_wq, B_wo)
```

```python
import contextlib

import jax
import jax.numpy as jnp
from jax import lax
import jax.experimental.pallas as pl
import jax.experimental.pallas.tpu as pltpu

B, Sq, D, H, Sk, Dh = 8, 160, 512, 32, 512, 128
LOG2E = 1.4426950408889634
SCALE = Dh ** -0.5
f32 = jnp.float32; bf16 = jnp.bfloat16
NH = 4
NHG = H // NH
NW = 2 * NHG
GW = NH * Dh

def make_v9(interpret=False, J=6, NS=3, LA=2, vmem=110, kv_pos=0.25, scopes=False, dbg_nokv=False, nb0=8):
    assert 2 <= J <= NHG and LA < NS and LA <= J
    def kernel(ax, ak, av, awq, awo, bx, bk, bv, bwq, bwo, out_hbm,
               x_buf, k_buf, v_buf, wq_buf, wo_buf, q_buf, acc, out_buf,
               x_sem, wq_sem, kv_sem, o_sem):
        def scope(name): return jax.named_scope(name) if scopes else contextlib.nullcontext()
        def slot_of(w):
            if isinstance(w, int): return w % NS
            return (w & (NS - 1)) if NS in (2, 4, 8) else lax.rem(w, NS)
        zero = pl.program_id(0)
        def cols(w):
            c0 = (w & (NHG - 1)) * GW
            return pl.ds(c0 if isinstance(c0, int) else pl.multiple_of(c0, GW), GW)
        def wq_copy(src, g, sem): return pltpu.make_async_copy(src.at[:, cols(g)], wq_buf.at[g], sem)
        def wo_copy(src, g, sem): return pltpu.make_async_copy(src.at[cols(g), :], wo_buf.at[g], sem)
        def kv_copies(kh, vh, w, sem):
            hg = w & (NHG - 1); slot = slot_of(w)
            if dbg_nokv: return []
            return [pltpu.make_async_copy(kh.at[:, pl.ds(hg * NH, NH)], k_buf.at[slot], sem),
                    pltpu.make_async_copy(vh.at[:, pl.ds(hg * NH, NH)], v_buf.at[slot], sem)]
        def when(cond):
            if isinstance(cond, bool):
                return (lambda f: f()) if cond else (lambda f: None)
            return pl.when(cond)
        def band(a, b):
            if isinstance(a, bool) and isinstance(b, bool): return a and b
            return a & b
        def start_piece(w):
            sem = kv_sem.at[slot_of(w) if not isinstance(w, int) else w % NS]
            @when(w < NHG)
            def _():
                for c in kv_copies(ak, av, w, sem) + [wo_copy(awo, w, sem)]: c.start()
            @when(band(w >= NHG, w < NW))
            def _():
                for c in kv_copies(bk, bv, w, sem) + [wo_copy(bwo, w, sem)]: c.start()
            @when(w + J < NHG)
            def _(): wq_copy(awq, w + J, sem).start()
            @when(band(w + J >= NHG, w + J < NW))
            def _(): wq_copy(bwq, w + J, sem).start()
        def wait_piece(w, with_q):
            sem = kv_sem.at[slot_of(w)]
            cps = kv_copies(ak, av, w, sem) + [wo_copy(awo, w, sem)]
            if with_q: cps.append(wq_copy(awq, w, sem))
            for c in cps: c.wait()
        NX = B // nb0
        def xa_copy(i, sem): return pltpu.make_async_copy(ax.at[pl.ds(i * nb0, nb0)], x_buf.at[0, pl.ds(i * nb0, nb0)], sem)
        def xb_copy(): return pltpu.make_async_copy(bx, x_buf.at[1], x_sem)
        def out_copy(blk, b):
            return pltpu.make_async_copy(out_buf.at[blk, b], out_hbm.at[b, :, pl.ds(pl.multiple_of(blk * D, D) if not isinstance(blk, int) else blk * D, D)], o_sem)
        def ordered(lo, hi, fn):
            lax.fori_loop(lo + zero, hi + zero, lambda i, c: (fn(i), c)[1], 0)

        with scope("prologue"):
            xa_copy(0, wq_sem.at[0]).start()
            wq_copy(awq, 0, wq_sem.at[0]).start()
            if NX > 1: ordered(1, NX, lambda i: xa_copy(i, wq_sem.at[i]).start())
            ordered(1, J, lambda g: wq_copy(awq, g, wq_sem.at[NX - 1 + g]).start())
            for w in range(LA):
                ordered(0, 1, lambda i, w=w: start_piece(w))
                if w == 0: ordered(0, 1, lambda i: xb_copy().start())
            acc[...] = jnp.zeros_like(acc)

        def q_proj(g, b, hi):
            blk = g >> 3
            t = jnp.dot(x_buf[blk, b], wq_buf[g, :, hi * Dh:(hi + 1) * Dh], preferred_element_type=f32)
            q_buf[g, b, :, hi * Dh:(hi + 1) * Dh] = (t * (SCALE * LOG2E)).astype(bf16)

        def q_step0(i, c):
            with scope("wait0"):
                xa_copy(i, wq_sem.at[i]).wait()
                @pl.when(i == 0)
                def _(): wq_copy(awq, 0, wq_sem.at[0]).wait()
            for b in range(nb0):
                for hi in range(NH): q_proj(0, i * nb0 + b, hi)
            return c
        def q_step(g, c):
            with scope("wait1"):
                if nb0 == B:
                    @pl.when(g == 0)
                    def _(): xa_copy(0, wq_sem.at[0]).wait()
                    wq_copy(awq, g, wq_sem.at[g]).wait()
                else:
                    wq_copy(awq, g, wq_sem.at[NX - 1 + g]).wait()
            for b in range(B):
                for hi in range(NH): q_proj(g, b, hi)
            return c
        with scope("ph1_Q"):
            if nb0 < B:
                lax.fori_loop(0, NX, q_step0, 0)
                lax.fori_loop(1, J, q_step, 0)
            else:
                lax.fori_loop(0, J, q_step, 0)
        xb_copy().wait()

        def att_step(w, with_q):
            slot = slot_of(w); blk = w >> 3
            with scope("wait2" if with_q else "wait3"):
                wait_piece(w, with_q)
            units = [(b, hi) for b in range(B) for hi in range(NH)]
            N = len(units)
            p, r, o, ocat = {}, {}, {}, {}
            def Sx(u):
                b, hi = units[u]
                sc = lax.dot_general(q_buf[w, b, :, hi * Dh:(hi + 1) * Dh], k_buf[slot, b, hi], (((1,), (1,)), ((), ())), preferred_element_type=f32)
                m = jnp.max(sc, axis=-1, keepdims=True)
                e = jnp.exp2(sc - m)
                l = jnp.sum(e, axis=-1, keepdims=True)
                p[u] = e.astype(bf16)
                rr = pl.reciprocal(l, approx=True)
                r[u] = rr * (2.0 - l * rr)
            def V(u):
                b, hi = units[u]
                t = jnp.dot(p.pop(u), v_buf[slot, b, hi], preferred_element_type=f32)
                o[u] = (t * r.pop(u)).astype(bf16)
            def O(grp, j):
                b, _ = units[grp]
                if grp not in ocat:
                    ocat[grp] = jnp.concatenate([o.pop(grp + i) for i in range(NH)], axis=-1)
                y = jnp.dot(ocat[grp], wo_buf[w, :, j * 128:(j + 1) * 128], preferred_element_type=f32)
                a = acc[blk, b, :, j * 128:(j + 1) * 128] + y
                acc[blk, b, :, j * 128:(j + 1) * 128] = a
                out_buf[blk, b, :, j * 128:(j + 1) * 128] = a.astype(bf16)
                if j == 3:
                    @pl.when((w & (NHG - 1)) == NHG - 1)
                    def _(): out_copy(blk, b).start()
            pend = []
            for u in range(N + 1):
                if u == int(kv_pos * N): start_piece(w + LA)
                if u < N: Sx(u)
                ready = []
                if u >= 1:
                    V(u - 1)
                    if (u - 1) % NH == NH - 1:
                        ready = [(u - NH, j) for j in range(4)]
                if with_q and u < N: q_proj(w + J, *units[u])
                if pend: O(*pend.pop(0))
                pend += ready
            while pend: O(*pend.pop(0))

        with scope("ph2_AttQ"):
            lax.fori_loop(0, NW - J, lambda w, c: (att_step(w, True), c)[1], 0)
        with scope("ph3_Att"):
            lax.fori_loop(NW - J, NW, lambda w, c: (att_step(w, False), c)[1], 0)

        with scope("epilogue"):
            for blk in range(2):
                for b in range(B):
                    out_copy(blk, b).wait()

    anys = pl.BlockSpec(memory_space=pl.ANY)
    @jax.jit
    def fn(*args):
        return pl.pallas_call(
            kernel, grid=(1,), in_specs=[anys] * 10, out_specs=anys,
            out_shape=jax.ShapeDtypeStruct((B, Sq, 2 * D), bf16),
            scratch_shapes=[
                pltpu.VMEM((2, B, Sq, D), bf16),
                pltpu.VMEM((NS, B, NH, Sk, Dh), bf16),
                pltpu.VMEM((NS, B, NH, Sk, Dh), bf16),
                pltpu.VMEM((NW, D, GW), bf16),
                pltpu.VMEM((NW, GW, D), bf16),
                pltpu.VMEM((NW, B, Sq, GW), bf16),
                pltpu.VMEM((2, B, Sq, D), f32),
                pltpu.VMEM((2, B, Sq, D), bf16),
                pltpu.SemaphoreType.DMA(()),
                pltpu.SemaphoreType.DMA((B + NHG,)),
                pltpu.SemaphoreType.DMA((NS,)),
                pltpu.SemaphoreType.DMA(()),
            ],
            compiler_params=pltpu.CompilerParams(vmem_limit_bytes=vmem * 1024 * 1024, disable_bounds_checks=True),
            interpret=interpret,
        )(*args)
    return fn


_impl = make_v9(J=5, nb0=2)


def pallas_concat_heads__mha_block_cached__mha_block_cached__near_ridge_kernel(
    A_x, A_k_cache, A_v_cache, A_wq, A_wo, B_x, B_k_cache, B_v_cache, B_wq, B_wo
):
    return _impl(A_x, A_k_cache, A_v_cache, A_wq, A_wo, B_x, B_k_cache, B_v_cache, B_wq, B_wo)
```

```python
import contextlib

import jax
import jax.numpy as jnp
from jax import lax
import jax.experimental.pallas as pl
import jax.experimental.pallas.tpu as pltpu

B, Sq, D, H, Sk, Dh = 8, 160, 512, 32, 512, 128
LOG2E = 1.4426950408889634
SCALE = Dh ** -0.5
f32 = jnp.float32; bf16 = jnp.bfloat16
NH = 4
NHG = H // NH
NW = 2 * NHG
GW = NH * Dh

def make_v9(interpret=False, J=6, NS=3, LA=2, vmem=110, kv_pos=0.25, scopes=False, dbg_nokv=False, nb0=8, q_first=False, vlag=1, xb_late=False, order='SVQO', segs=None, qloop=None):
    assert 2 <= J <= NHG and LA < NS and LA <= J
    def kernel(ax, ak, av, awq, awo, bx, bk, bv, bwq, bwo, out_hbm,
               x_buf, k_buf, v_buf, wq_buf, wo_buf, q_buf, acc, out_buf,
               x_sem, wq_sem, kv_sem, o_sem):
        def scope(name): return jax.named_scope(name) if scopes else contextlib.nullcontext()
        def slot_of(w):
            if isinstance(w, int): return w % NS
            return (w & (NS - 1)) if NS in (2, 4, 8) else lax.rem(w, NS)
        zero = pl.program_id(0)
        def cols(w):
            c0 = (w & (NHG - 1)) * GW
            return pl.ds(c0 if isinstance(c0, int) else pl.multiple_of(c0, GW), GW)
        def wq_copy(src, g, sem): return pltpu.make_async_copy(src.at[:, cols(g)], wq_buf.at[g], sem)
        def wo_copy(src, g, sem): return pltpu.make_async_copy(src.at[cols(g), :], wo_buf.at[g], sem)
        def kv_copies(kh, vh, w, sem):
            hg = w & (NHG - 1); slot = slot_of(w)
            if dbg_nokv: return []
            return [pltpu.make_async_copy(kh.at[:, pl.ds(hg * NH, NH)], k_buf.at[slot], sem),
                    pltpu.make_async_copy(vh.at[:, pl.ds(hg * NH, NH)], v_buf.at[slot], sem)]
        def when(cond):
            if isinstance(cond, bool):
                return (lambda f: f()) if cond else (lambda f: None)
            return pl.when(cond)
        def band(a, b):
            if isinstance(a, bool) and isinstance(b, bool): return a and b
            return a & b
        def start_piece(w):
            sem = kv_sem.at[slot_of(w) if not isinstance(w, int) else w % NS]
            @when(w < NHG)
            def _():
                for c in kv_copies(ak, av, w, sem) + [wo_copy(awo, w, sem)]: c.start()
            @when(band(w >= NHG, w < NW))
            def _():
                for c in kv_copies(bk, bv, w, sem) + [wo_copy(bwo, w, sem)]: c.start()
            @when(w + J < NHG)
            def _(): wq_copy(awq, w + J, sem).start()
            @when(band(w + J >= NHG, w + J < NW))
            def _(): wq_copy(bwq, w + J, sem).start()
        def wait_piece(w, with_q):
            sem = kv_sem.at[slot_of(w)]
            cps = kv_copies(ak, av, w, sem) + [wo_copy(awo, w, sem)]
            if with_q: cps.append(wq_copy(awq, w, sem))
            for c in cps: c.wait()
        NX = B // nb0
        def xa_copy(i, sem): return pltpu.make_async_copy(ax.at[pl.ds(i * nb0, nb0)], x_buf.at[0, pl.ds(i * nb0, nb0)], sem)
        def xb_copy(): return pltpu.make_async_copy(bx, x_buf.at[1], x_sem)
        def out_copy(blk, b):
            return pltpu.make_async_copy(out_buf.at[blk, b], out_hbm.at[b, :, pl.ds(pl.multiple_of(blk * D, D) if not isinstance(blk, int) else blk * D, D)], o_sem)
        def ordered(lo, hi, fn):
            lax.fori_loop(lo + zero, hi + zero, lambda i, c: (fn(i), c)[1], 0)

        def seg_copies(i):
            g0, g1, b0, b1 = segs[i]
            sem = wq_sem.at[i]
            cps = []
            if g0 == 0:
                cps.append(pltpu.make_async_copy(ax.at[pl.ds(b0, b1 - b0)], x_buf.at[0, pl.ds(b0, b1 - b0)], sem))
            if b0 == 0:
                cps += [wq_copy(awq, g, sem) for g in range(g0, g1)]
            return cps

        with scope("prologue"):
            if segs is None:
                xa_copy(0, wq_sem.at[0]).start()
                wq_copy(awq, 0, wq_sem.at[0]).start()
                if NX > 1: ordered(1, NX, lambda i: xa_copy(i, wq_sem.at[i]).start())
                ordered(1, J, lambda g: wq_copy(awq, g, wq_sem.at[NX - 1 + g]).start())
            else:
                for c in seg_copies(0): c.start()
                for i in range(1, len(segs)):
                    ordered(0, 1, lambda _, i=i: [c.start() for c in seg_copies(i)])
                gl = segs[-1][1]
                if gl < J:
                    ordered(0, (J - gl) // qloop, lambda it: [wq_copy(awq, gl + it * qloop + k, wq_sem.at[len(segs) + it]).start() for k in range(qloop)])
            for w in range(LA):
                ordered(0, 1, lambda i, w=w: start_piece(w))
                if w == (LA - 1 if xb_late else 0): ordered(0, 1, lambda i: xb_copy().start())
            acc[...] = jnp.zeros_like(acc)

        def q_proj(g, b, hi):
            blk = g >> 3
            t = jnp.dot(x_buf[blk, b], wq_buf[g, :, hi * Dh:(hi + 1) * Dh], preferred_element_type=f32)
            q_buf[g, b, :, hi * Dh:(hi + 1) * Dh] = (t * (SCALE * LOG2E)).astype(bf16)

        def q_step0(i, c):
            with scope("wait0"):
                xa_copy(i, wq_sem.at[i]).wait()
                @pl.when(i == 0)
                def _(): wq_copy(awq, 0, wq_sem.at[0]).wait()
            for b in range(nb0):
                for hi in range(NH): q_proj(0, i * nb0 + b, hi)
            return c
        def q_step(g, c):
            with scope("wait1"):
                if nb0 == B:
                    @pl.when(g == 0)
                    def _(): xa_copy(0, wq_sem.at[0]).wait()
                    wq_copy(awq, g, wq_sem.at[g]).wait()
                else:
                    wq_copy(awq, g, wq_sem.at[NX - 1 + g]).wait()
            for b in range(B):
                for hi in range(NH): q_proj(g, b, hi)
            return c
        with scope("ph1_Q"):
            if segs is not None:
                gl = segs[-1][1]
                assert segs[0][0] == 0 and (gl == J or (J - gl) % qloop == 0)
                for i, (g0, g1, b0, b1) in enumerate(segs):
                    for c in seg_copies(i): c.wait()
                    for g in range(g0, g1):
                        for b in range(b0, b1):
                            for hi in range(NH): q_proj(g, b, hi)
                if gl < J:
                    def q_iter(it, c):
                        g0 = gl + it * qloop
                        for k in range(qloop): wq_copy(awq, g0 + k, wq_sem.at[len(segs) + it]).wait()
                        for k in range(qloop):
                            for b in range(B):
                                for hi in range(NH): q_proj(g0 + k, b, hi)
                        return c
                    lax.fori_loop(0, (J - gl) // qloop, q_iter, 0)
            elif nb0 < B:
                lax.fori_loop(0, NX, q_step0, 0)
                lax.fori_loop(1, J, q_step, 0)
            else:
                lax.fori_loop(0, J, q_step, 0)
        if not xb_late: xb_copy().wait()

        def att_step(w, with_q):
            slot = slot_of(w); blk = w >> 3
            with scope("wait2" if with_q else "wait3"):
                wait_piece(w, with_q)
                if xb_late and with_q:
                    if NHG - J <= 0: raise ValueError
                    @pl.when(w == NHG - J)
                    def _(): xb_copy().wait()
            units = [(b, hi) for b in range(B) for hi in range(NH)]
            N = len(units)
            p, r, o, ocat = {}, {}, {}, {}
            def Sx(u):
                b, hi = units[u]
                sc = lax.dot_general(q_buf[w, b, :, hi * Dh:(hi + 1) * Dh], k_buf[slot, b, hi], (((1,), (1,)), ((), ())), preferred_element_type=f32)
                m = jnp.max(sc, axis=-1, keepdims=True)
                e = jnp.exp2(sc - m)
                l = jnp.sum(e, axis=-1, keepdims=True)
                p[u] = e.astype(bf16)
                rr = pl.reciprocal(l, approx=True)
                r[u] = rr * (2.0 - l * rr)
            def V(u):
                b, hi = units[u]
                t = jnp.dot(p.pop(u), v_buf[slot, b, hi], preferred_element_type=f32)
                o[u] = (t * r.pop(u)).astype(bf16)
            def O(grp, j):
                b, _ = units[grp]
                if grp not in ocat:
                    ocat[grp] = jnp.concatenate([o.pop(grp + i) for i in range(NH)], axis=-1)
                y = jnp.dot(ocat[grp], wo_buf[w, :, j * 128:(j + 1) * 128], preferred_element_type=f32)
                a = acc[blk, b, :, j * 128:(j + 1) * 128] + y
                acc[blk, b, :, j * 128:(j + 1) * 128] = a
                out_buf[blk, b, :, j * 128:(j + 1) * 128] = a.astype(bf16)
                if j == 3:
                    @pl.when((w & (NHG - 1)) == NHG - 1)
                    def _(): out_copy(blk, b).start()
            pend = []
            qn = 0
            if with_q and q_first:
                q_proj(w + J, *units[0]); qn = 1
            for u in range(N + vlag):
                if u == int(kv_pos * N): start_piece(w + LA)
                ready = []
                for ch in order:
                    if ch == 'S':
                        if u < N: Sx(u)
                    elif ch == 'V':
                        if u >= vlag:
                            V(u - vlag)
                            if (u - vlag) % NH == NH - 1:
                                ready = [(u - vlag - (NH - 1), j) for j in range(4)]
                    elif ch == 'Q':
                        if with_q and qn < N and u < N:
                            q_proj(w + J, *units[qn]); qn += 1
                    elif ch == 'O':
                        if pend: O(*pend.pop(0))
                pend += ready
            while pend: O(*pend.pop(0))
            assert qn == (N if with_q else 0)

        with scope("ph2_AttQ"):
            lax.fori_loop(0, NW - J, lambda w, c: (att_step(w, True), c)[1], 0)
        with scope("ph3_Att"):
            lax.fori_loop(NW - J, NW, lambda w, c: (att_step(w, False), c)[1], 0)

        with scope("epilogue"):
            for blk in range(2):
                for b in range(B):
                    out_copy(blk, b).wait()

    anys = pl.BlockSpec(memory_space=pl.ANY)
    @jax.jit
    def fn(*args):
        return pl.pallas_call(
            kernel, grid=(1,), in_specs=[anys] * 10, out_specs=anys,
            out_shape=jax.ShapeDtypeStruct((B, Sq, 2 * D), bf16),
            scratch_shapes=[
                pltpu.VMEM((2, B, Sq, D), bf16),
                pltpu.VMEM((NS, B, NH, Sk, Dh), bf16),
                pltpu.VMEM((NS, B, NH, Sk, Dh), bf16),
                pltpu.VMEM((NW, D, GW), bf16),
                pltpu.VMEM((NW, GW, D), bf16),
                pltpu.VMEM((NW, B, Sq, GW), bf16),
                pltpu.VMEM((2, B, Sq, D), f32),
                pltpu.VMEM((2, B, Sq, D), bf16),
                pltpu.SemaphoreType.DMA(()),
                pltpu.SemaphoreType.DMA((B + NHG,)),
                pltpu.SemaphoreType.DMA((NS,)),
                pltpu.SemaphoreType.DMA(()),
            ],
            compiler_params=pltpu.CompilerParams(vmem_limit_bytes=vmem * 1024 * 1024, disable_bounds_checks=True),
            interpret=interpret,
        )(*args)
    return fn


_impl = make_v9(J=5, q_first=True, NS=4, xb_late=True, vlag=2, segs=((0,1,0,1),(0,1,1,3),(0,1,3,8)), qloop=2)


def pallas_concat_heads__mha_block_cached__mha_block_cached__near_ridge_kernel(
    A_x, A_k_cache, A_v_cache, A_wq, A_wo, B_x, B_k_cache, B_v_cache, B_wq, B_wo
):
    return _impl(A_x, A_k_cache, A_v_cache, A_wq, A_wo, B_x, B_k_cache, B_v_cache, B_wq, B_wo)
```

```python
import jax
import jax.numpy as jnp
from jax import lax
import jax.experimental.pallas as pl
import jax.experimental.pallas.tpu as pltpu

B, Sq, D, H, Sk, Dh = 8, 160, 512, 32, 512, 128
NH = 4
NHG = H // NH
NW = 2 * NHG
GW = NH * Dh
J = 5
NS = 4
LA = 2
VLAG = 3
Q_SEGS = ((0, 1), (1, 3), (3, 8))
Q_LOOP = 2
C = (Dh ** -0.5) * 1.4426950408889634

f32, bf16 = jnp.float32, jnp.bfloat16


def _kernel(ax, ak, av, awq, awo, bx, bk, bv, bwq, bwo, out_hbm,
            x_buf, k_buf, v_buf, wq_buf, wo_buf, q_buf, acc, out_buf,
            xb_sem, q_sem, kv_sem, o_sem):
    zero = pl.program_id(0)

    def ordered(lo, hi, fn):
        def body(i, c):
            fn(i)
            return c
        lax.fori_loop(lo + zero, hi + zero, body, 0)

    def when(cond):
        if isinstance(cond, bool):
            return (lambda f: f()) if cond else (lambda f: None)
        return pl.when(cond)

    def cols(g):
        c0 = (g & (NHG - 1)) * GW
        return pl.ds(c0 if isinstance(c0, int) else pl.multiple_of(c0, GW), GW)

    def wq_copy(src, g, sem):
        return pltpu.make_async_copy(src.at[:, cols(g)], wq_buf.at[g], sem)

    def wo_copy(src, g, sem):
        return pltpu.make_async_copy(src.at[cols(g), :], wo_buf.at[g], sem)

    def x_copy(src, blk, b0, b1, sem):
        return pltpu.make_async_copy(src.at[pl.ds(b0, b1 - b0)], x_buf.at[blk, pl.ds(b0, b1 - b0)], sem)

    def att_copies(kh, vh, woh, w):
        slot = w & (NS - 1)
        sem = kv_sem.at[slot]
        heads = pl.ds((w & (NHG - 1)) * NH, NH)
        return [pltpu.make_async_copy(kh.at[:, heads], k_buf.at[slot], sem),
                pltpu.make_async_copy(vh.at[:, heads], v_buf.at[slot], sem),
                wo_copy(woh, w, sem)]

    def start_piece(w):
        sem = kv_sem.at[w & (NS - 1)]

        @when(w < NHG)
        def _():
            for c in att_copies(ak, av, awo, w):
                c.start()

        @when((w >= NHG) & (w < NW))
        def _():
            for c in att_copies(bk, bv, bwo, w):
                c.start()

        @when(w + J < NHG)
        def _():
            wq_copy(awq, w + J, sem).start()

        @when((w + J >= NHG) & (w + J < NW))
        def _():
            wq_copy(bwq, w + J, sem).start()

    def wait_piece(w, with_q):
        cps = att_copies(ak, av, awo, w)
        if with_q:
            cps.append(wq_copy(awq, w + J, kv_sem.at[w & (NS - 1)]))
        for c in cps:
            c.wait()

    def seg_copies(i):
        b0, b1 = Q_SEGS[i]
        cps = [x_copy(ax, 0, b0, b1, q_sem.at[i])]
        if i == 0:
            cps.append(wq_copy(awq, 0, q_sem.at[0]))
        return cps

    def qloop_copies(it):
        return [wq_copy(awq, 1 + it * Q_LOOP + k, q_sem.at[len(Q_SEGS) + it]) for k in range(Q_LOOP)]

    def out_copy(blk, b, j):
        c0 = pl.multiple_of(blk * D + j * 128, 128)
        return pltpu.make_async_copy(out_buf.at[blk, b, :, pl.ds(j * 128, 128)],
                                     out_hbm.at[b, :, pl.ds(c0, 128)], o_sem)

    n_qloop = (J - 1) // Q_LOOP

    for c in seg_copies(0):
        c.start()
    for i in range(1, len(Q_SEGS)):
        ordered(0, 1, lambda _, i=i: [c.start() for c in seg_copies(i)])
    ordered(0, n_qloop, lambda it: [c.start() for c in qloop_copies(it)])
    for w in range(LA):
        ordered(0, 1, lambda _, w=w: start_piece(w))
    ordered(0, 1, lambda _: x_copy(bx, 1, 0, B, xb_sem).start())
    acc[...] = jnp.zeros_like(acc)

    def q_proj(g, b, hi):
        t = jnp.dot(x_buf[g >> 3, b], wq_buf[g, :, hi * Dh:(hi + 1) * Dh], preferred_element_type=f32)
        q_buf[g, b, :, hi * Dh:(hi + 1) * Dh] = (t * C).astype(bf16)

    for i, (b0, b1) in enumerate(Q_SEGS):
        for c in seg_copies(i):
            c.wait()
        for b in range(b0, b1):
            for hi in range(NH):
                q_proj(0, b, hi)

    def q_iter(it, carry):
        for c in qloop_copies(it):
            c.wait()
        for k in range(Q_LOOP):
            for b in range(B):
                for hi in range(NH):
                    q_proj(1 + it * Q_LOOP + k, b, hi)
        return carry

    lax.fori_loop(0, n_qloop, q_iter, 0)

    def att_step(w, with_q):
        slot = w & (NS - 1)
        blk = w >> 3
        wait_piece(w, with_q)
        if with_q:
            @pl.when(w == NHG - J)
            def _():
                x_copy(bx, 1, 0, B, xb_sem).wait()

        units = [(b, hi) for b in range(B) for hi in range(NH)]
        n_units = len(units)
        p, r, o, ocat = {}, {}, {}, {}

        def job_s(u):
            b, hi = units[u]
            s = lax.dot_general(q_buf[w, b, :, hi * Dh:(hi + 1) * Dh], k_buf[slot, b, hi],
                                (((1,), (1,)), ((), ())), preferred_element_type=f32)
            m = jnp.max(s, axis=-1, keepdims=True)
            e = jnp.exp2(s - m)
            l = jnp.sum(e, axis=-1, keepdims=True)
            p[u] = e.astype(bf16)
            rr = pl.reciprocal(l, approx=True)
            r[u] = rr * (2.0 - l * rr)

        def job_v(u):
            b, hi = units[u]
            t = jnp.dot(p.pop(u), v_buf[slot, b, hi], preferred_element_type=f32)
            o[u] = (t * r.pop(u)).astype(bf16)

        def job_o(grp, j):
            b = units[grp][0]
            if grp not in ocat:
                ocat[grp] = jnp.concatenate([o.pop(grp + i) for i in range(NH)], axis=-1)
            cs = slice(j * 128, (j + 1) * 128)
            y = jnp.dot(ocat[grp], wo_buf[w, :, cs], preferred_element_type=f32)
            a = acc[blk, b, :, cs] + y
            acc[blk, b, :, cs] = a
            out_buf[blk, b, :, cs] = a.astype(bf16)

            @pl.when((w & (NHG - 1)) == NHG - 1)
            def _():
                out_copy(blk, b, j).start()

        pending = []
        q_next = 0
        if with_q:
            q_proj(w + J, *units[0])
            q_next = 1
        for u in range(n_units + VLAG):
            if u == n_units // 4:
                start_piece(w + LA)
            if u < n_units:
                job_s(u)
            ready = []
            if u >= VLAG:
                job_v(u - VLAG)
                if (u - VLAG) % NH == NH - 1:
                    ready = [(u - VLAG - (NH - 1), j) for j in range(D // 128)]
            if with_q and q_next < n_units:
                q_proj(w + J, *units[q_next])
                q_next += 1
            if pending:
                job_o(*pending.pop(0))
            pending += ready
        while pending:
            job_o(*pending.pop(0))

    lax.fori_loop(0, NW - J, lambda w, c: (att_step(w, True), c)[1], 0)
    lax.fori_loop(NW - J, NW, lambda w, c: (att_step(w, False), c)[1], 0)

    pltpu.make_async_copy(out_buf, out_buf, o_sem).wait()


@jax.jit
def pallas_concat_heads__mha_block_cached__mha_block_cached__near_ridge_kernel(
    A_x: jax.Array,
    A_k_cache: jax.Array,
    A_v_cache: jax.Array,
    A_wq: jax.Array,
    A_wo: jax.Array,
    B_x: jax.Array,
    B_k_cache: jax.Array,
    B_v_cache: jax.Array,
    B_wq: jax.Array,
    B_wo: jax.Array,
):
    hbm = pl.BlockSpec(memory_space=pl.ANY)
    return pl.pallas_call(
        _kernel,
        grid=(1,),
        in_specs=[hbm] * 10,
        out_specs=hbm,
        out_shape=jax.ShapeDtypeStruct((B, Sq, 2 * D), bf16),
        scratch_shapes=[
            pltpu.VMEM((2, B, Sq, D), bf16),
            pltpu.VMEM((NS, B, NH, Sk, Dh), bf16),
            pltpu.VMEM((NS, B, NH, Sk, Dh), bf16),
            pltpu.VMEM((NW, D, GW), bf16),
            pltpu.VMEM((NW, GW, D), bf16),
            pltpu.VMEM((NW, B, Sq, GW), bf16),
            pltpu.VMEM((2, B, Sq, D), f32),
            pltpu.VMEM((2, B, Sq, D), bf16),
            pltpu.SemaphoreType.DMA(()),
            pltpu.SemaphoreType.DMA((len(Q_SEGS) + (J - 1) // Q_LOOP,)),
            pltpu.SemaphoreType.DMA((NS,)),
            pltpu.SemaphoreType.DMA(()),
        ],
        compiler_params=pltpu.CompilerParams(
            dimension_semantics=("arbitrary",),
            vmem_limit_bytes=110 * 1024 * 1024,
            disable_bounds_checks=True,
        ),
    )(A_x, A_k_cache, A_v_cache, A_wq, A_wo, B_x, B_k_cache, B_v_cache, B_wq, B_wo)
```
